```python
import os as _os
_os.environ.setdefault('JAX_PLATFORMS', 'cpu')
import jax
import jax.numpy as jnp

def _softmax(x, axis=-1):
    return jax.nn.softmax(x, axis=axis)

def _gelu(x):
    return jax.nn.gelu(x, approximate=True)

def _silu(x):
    return jax.nn.silu(x)

def _sigmoid(x):
    return jax.nn.sigmoid(x)

def _layernorm(x, axis=-1, eps=1e-05):
    m = jnp.mean(x, axis=axis, keepdims=True)
    v = jnp.var(x, axis=axis, keepdims=True)
    return (x - m) / jnp.sqrt(v + eps)

def _scatter_add(tgt, idx, src, axis=0):
    return tgt.at[idx].add(src)

def _segment_sum(src, seg, n):
    return jax.ops.segment_sum(src, seg, n)

class _Rng:

    def __init__(self, key):
        self._k = key

    def _next(self):
        self._k, sub = jax.random.split(self._k)
        return sub

    def normal(self, shape):
        return jax.random.normal(self._next(), shape, dtype=jnp.bfloat16)

    def randint(self, lo, hi, shape):
        return jax.random.randint(self._next(), shape, lo, hi, dtype=jnp.int32)

    def uniform(self, shape, lo=0.0, hi=1.0):
        return jax.random.uniform(self._next(), shape, jnp.bfloat16, lo, hi)

    def permutation(self, n):
        return jax.random.permutation(self._next(), n)
kernel_name = 'parallel_sum__memory_aug_recurrent_mem_tr__dense_activation_gelu__prompt'

def setup_inputs():
    _rng = _Rng(jax.random.key(int.from_bytes(__import__("os").urandom(4), "little")))
    _w = lambda a: (lambda t: t.astype(jnp.bfloat16) if jnp.issubdtype(t.dtype, jnp.floating) else t)(jnp.asarray(a))

    def _A_setup():
        B, S, Dm = (1, 2048, 1024)
        H, Dh = (32, 128)
        M, seg = (8, 32)
        seg = min(seg, S)
        S = S // seg * seg
        return {'x': _w((lambda *s: _rng.normal(s) * 0.05)(B, S, Dm)), 'mem0': _w((lambda *s: _rng.normal(s) * 0.2)(B, M, Dm)), 'Wq': _w((lambda *s: _rng.normal(s) * 0.8)(Dm, H, Dh) * Dm ** (-0.5)), 'Wk': _w((lambda *s: _rng.normal(s) * 0.8)(Dm, H, Dh) * Dm ** (-0.5)), 'Wv': _w((lambda *s: _rng.normal(s) * 0.2)(Dm, H, Dh) * Dm ** (-0.5)), 'Wo': _w((lambda *s: _rng.normal(s) * 0.2)(H, Dh, Dm) * (H * Dh) ** (-0.5)), 'seg_len': seg}
    _A_in = _A_setup()

    def _B_setup():
        B, S, D, F = (1, 2048, 1024, 3584)
        return {'x': _w((lambda *s: _rng.normal(s) * 0.05)(B, S, D)), 'w1': _w((lambda *s: _rng.normal(s) * 0.1)(D, F) * D ** (-0.5)), 'b1': _w((lambda *s: _rng.normal(s) * 0.1)(F) * 0.01), 'w2': _w((lambda *s: _rng.normal(s) * 0.1)(F, D) * F ** (-0.5)), 'b2': _w((lambda *s: _rng.normal(s) * 0.05)(D) * 0.01)}
    _B_in = _B_setup()
    return {'A_x': _A_in['x'], 'A_mem0': _A_in['mem0'], 'A_Wq': _A_in['Wq'], 'A_Wk': _A_in['Wk'], 'A_Wv': _A_in['Wv'], 'A_Wo': _A_in['Wo'], 'A_seg_len': _A_in['seg_len'], 'B_x': _B_in['x'], 'B_w1': _B_in['w1'], 'B_b1': _B_in['b1'], 'B_w2': _B_in['w2'], 'B_b2': _B_in['b2']}

def reference(A_x, A_mem0, A_Wq, A_Wk, A_Wv, A_Wo, A_seg_len, B_x, B_w1, B_b1, B_w2, B_b2):

    def _A_ref(x, mem0, Wq, Wk, Wv, Wo, seg_len):
        B, S, Dm = x.shape
        H, Dh = (Wq.shape[1], Wq.shape[2])
        M = mem0.shape[1]
        scale = Dh ** (-0.5)
        n_seg = S // seg_len
        L = M + seg_len
        idx = jnp.arange(L)
        mask = (idx[:, None] < M) | (idx[:, None] >= idx[None, :])
        mem = mem0
        outs = []
        for s in range(n_seg):
            xs = x[:, s * seg_len:(s + 1) * seg_len, :].copy()
            h = jnp.concatenate([mem, xs], axis=1)
            q = jnp.einsum('btd,dhe->bhte', h, Wq)
            k = jnp.einsum('btd,dhe->bhte', h, Wk)
            v = jnp.einsum('btd,dhe->bhte', h, Wv)
            scores = jnp.einsum('bhqe,bhke->bhqk', q, k) * scale
            scores = jnp.where(mask[None, None], scores, -1000000000.0)
            p = _softmax(scores, axis=-1)
            o = jnp.einsum('bhqk,bhke->bhqe', p, v)
            o = jnp.einsum('bhte,hed->btd', o, Wo)
            mem = o[:, :M, :].copy()
            outs.append(o[:, M:, :])
        return jnp.concatenate(outs, axis=1)

    def _B_ref(x, w1, b1, w2, b2):
        h = jnp.einsum('bsd,df->bsf', x, w1) + b1
        h = _gelu(h)
        return jnp.einsum('bsf,fd->bsd', h, w2) + b2
    x = A_x
    xn = _layernorm(x, axis=-1)
    return x + _A_ref(xn, A_mem0, A_Wq, A_Wk, A_Wv, A_Wo, A_seg_len) + _B_ref(xn, B_w1, B_b1, B_w2, B_b2)
```

```python
import functools
import jax
import jax.numpy as jnp
from jax import lax
import jax.experimental.pallas as pl
import jax.experimental.pallas.tpu as pltpu

S = 2048
D = 1024
H = 32
DH = 128
MEM = 8
SEG = 32
FF = 3584
L = SEG + MEM
TB = 256
NB = S // TB
FC = 512
EPS = 1e-5
NP_O = D // DH
RCH = 16
f32 = jnp.float32
bf16 = jnp.bfloat16

SEM_X = 0
SEM_W1 = 8
SEM_W2 = 9
SEM_QKV = 10
SEM_WO = 13
SEM_OUT = 21
NSEM = 22


def _kernel(x_hbm, mem0_ref, wq_hbm, wk_hbm, wv_hbm, wo_hbm, w1_hbm, b1_ref, w2_hbm, b2_ref,
            out_hbm,
            x_scr, xn_scr, acc_scr, out_scr, w1_scr, w2_scr, stage, wp_scr, wo_scr,
            h_scr, q_scr, k_scr, v_scr, o_scr, sems):
    def x_copy(b):
        return pltpu.make_async_copy(x_hbm.at[pl.ds(b * TB, TB)], x_scr.at[pl.ds(b * TB, TB)], sems.at[SEM_X + b])

    w1_copy = pltpu.make_async_copy(w1_hbm, w1_scr, sems.at[SEM_W1])
    w2_copy = pltpu.make_async_copy(w2_hbm, w2_scr, sems.at[SEM_W2])
    qkv_hbm = (wq_hbm, wk_hbm, wv_hbm)

    def qkv_copy(m):
        return pltpu.make_async_copy(qkv_hbm[m], stage.at[m], sems.at[SEM_QKV + m])

    def wo_copy(j):
        return pltpu.make_async_copy(wo_hbm.at[:, pl.ds(j * DH, DH)], wo_scr.at[j], sems.at[SEM_WO + j])

    x_copy(0).start()
    w1_copy.start()
    w2_copy.start()
    for b in range(1, NB):
        x_copy(b).start()
    for m in range(3):
        qkv_copy(m).start()
    for j in range(NP_O):
        wo_copy(j).start()

    w1_copy.wait()
    w2_copy.wait()

    def ffn_body(b, carry):
        r0 = pl.multiple_of(b * TB, TB)
        pltpu.make_async_copy(x_hbm.at[pl.ds(r0, TB)], x_scr.at[pl.ds(r0, TB)], sems.at[SEM_X + b]).wait()
        x = x_scr[pl.ds(r0, TB), :].astype(f32)
        mu = jnp.mean(x, axis=-1, keepdims=True)
        xc = x - mu
        var = jnp.mean(xc * xc, axis=-1, keepdims=True)
        xn = (xc * lax.rsqrt(var + EPS)).astype(bf16)
        xn_scr[pl.ds(r0, TB), :] = xn
        acc = x + b2_ref[...].astype(f32)
        for c in range(FF // FC):
            h1 = jnp.dot(xn, w1_scr[:, c * FC:(c + 1) * FC], preferred_element_type=f32)
            h1 = h1 + b1_ref[:, c * FC:(c + 1) * FC].astype(f32)
            g = jax.nn.gelu(h1, approximate=True).astype(bf16)
            acc = acc + jnp.dot(g, w2_scr[c * FC:(c + 1) * FC, :], preferred_element_type=f32)
        acc_scr[pl.ds(r0, TB), :] = acc
        return carry

    lax.fori_loop(0, NB, ffn_body, 0)

    for m in range(3):
        qkv_copy(m).wait()

        def relayout(c, carry, m=m):
            d0 = pl.multiple_of(c * RCH, RCH)
            blk = stage[m, pl.ds(d0, RCH)]
            wp_scr[pl.ds(m * H, H), pl.ds(d0, RCH), :] = jnp.transpose(blk, (1, 0, 2))
            return carry

        lax.fori_loop(0, D // RCH, relayout, 0)
    for j in range(NP_O):
        wo_copy(j).wait()

    qi = lax.broadcasted_iota(jnp.int32, (L, L), 0)
    kj = lax.broadcasted_iota(jnp.int32, (L, L), 1)
    mask = (qi >= SEG) | (kj >= SEG) | (kj <= qi)
    scale = DH ** -0.5
    h_scr[SEG:L, :] = mem0_ref[...]

    def out_copy(r0):
        return pltpu.make_async_copy(out_scr.at[pl.ds(r0, SEG)], out_hbm.at[pl.ds(r0, SEG)], sems.at[SEM_OUT])

    def seg_body(s, carry):
        r0 = pl.multiple_of(s * SEG, SEG)
        h_scr[0:SEG, :] = xn_scr[pl.ds(r0, SEG), :]
        h = h_scr[...]
        for hd in range(H):
            q_scr[hd] = jnp.dot(h, wp_scr[hd], preferred_element_type=f32).astype(bf16)
            k_scr[hd] = jnp.dot(h, wp_scr[H + hd], preferred_element_type=f32).astype(bf16)
            v_scr[hd] = jnp.dot(h, wp_scr[2 * H + hd], preferred_element_type=f32).astype(bf16)
        q = q_scr[...]
        k = k_scr[...]
        v = v_scr[...]
        sc = jnp.einsum('hqd,hkd->hqk', q, k, preferred_element_type=f32) * scale
        sc = jnp.where(mask[None], sc, -1e9)
        m = jnp.max(sc, axis=-1, keepdims=True)
        e = jnp.exp(sc - m)
        l = jnp.sum(e, axis=-1, keepdims=True)
        p = (e / l).astype(bf16)
        oh = jnp.einsum('hqk,hkd->hqd', p, v, preferred_element_type=f32).astype(bf16)
        for hd in range(H):
            o_scr[:, hd * DH:(hd + 1) * DH] = oh[hd]
        o = o_scr[...]
        for j in range(NP_O):
            r = jnp.dot(o, wo_scr[j], preferred_element_type=f32)
            fin = acc_scr[pl.ds(r0, SEG), j * DH:(j + 1) * DH] + r[0:SEG]
            out_scr[pl.ds(r0, SEG), j * DH:(j + 1) * DH] = fin.astype(bf16)
            h_scr[SEG:L, j * DH:(j + 1) * DH] = r[SEG:L].astype(bf16)
        out_copy(r0).start()
        return carry

    lax.fori_loop(0, S // SEG, seg_body, 0)

    def wait_body(s, carry):
        out_copy(pl.multiple_of(s * SEG, SEG)).wait()
        return carry

    lax.fori_loop(0, S // SEG, wait_body, 0)


@jax.jit
def pallas_parallel_sum__memory_aug_recurrent_mem_tr__dense_activation_gelu__prompt_kernel(A_x, A_mem0, A_Wq, A_Wk, A_Wv, A_Wo, A_seg_len, B_x, B_w1, B_b1, B_w2, B_b2):
    del A_seg_len, B_x
    x = A_x.reshape(S, D)
    mem0 = A_mem0.reshape(MEM, D)
    wo = A_Wo.reshape(H * DH, D)
    b1 = B_b1.reshape(1, FF)
    b2 = B_b2.reshape(1, D)
    any_spec = pl.BlockSpec(memory_space=pl.ANY)
    vmem_spec = pl.BlockSpec(memory_space=pltpu.VMEM)
    out = pl.pallas_call(
        _kernel,
        out_shape=jax.ShapeDtypeStruct((S, D), bf16),
        in_specs=[any_spec, vmem_spec, any_spec, any_spec, any_spec, any_spec, any_spec, vmem_spec, any_spec, vmem_spec],
        out_specs=any_spec,
        scratch_shapes=[
            pltpu.VMEM((S, D), bf16),
            pltpu.VMEM((S, D), bf16),
            pltpu.VMEM((S, D), f32),
            pltpu.VMEM((S, D), bf16),
            pltpu.VMEM((D, FF), bf16),
            pltpu.VMEM((FF, D), bf16),
            pltpu.VMEM((3, D, H, DH), bf16),
            pltpu.VMEM((3 * H, D, DH), bf16),
            pltpu.VMEM((NP_O, H * DH, DH), bf16),
            pltpu.VMEM((L, D), bf16),
            pltpu.VMEM((H, L, DH), bf16),
            pltpu.VMEM((H, L, DH), bf16),
            pltpu.VMEM((H, L, DH), bf16),
            pltpu.VMEM((L, H * DH), bf16),
            pltpu.SemaphoreType.DMA((NSEM,)),
        ],
        compiler_params=pltpu.CompilerParams(
            vmem_limit_bytes=120 * 1024 * 1024,
        ),
    )(x, mem0, A_Wq, A_Wk, A_Wv, wo, B_w1, b1, B_w2, b2)
    return out.reshape(1, S, D)
```

```python
import jax
import jax.numpy as jnp
from jax import lax
import jax.experimental.pallas as pl
import jax.experimental.pallas.tpu as pltpu

S = 2048
D = 1024
H = 32
DH = 128
MEM = 8
SEG = 32
FF = 3584
L = SEG + MEM
TB = 256
NB = S // TB
RB = 512
NBB = S // RB
XPB = RB // TB
FC = 512
NFC = FF // FC
N_IT = NFC * NBB
N_IT1 = 12
RSTEPS = 3 * (D // 16) // (N_IT - N_IT1)
EPS = 1e-5
NP_O = D // DH
RCH = 16
f32 = jnp.float32
bf16 = jnp.bfloat16

SEM_X = 0
SEM_W1 = 8
SEM_W2 = SEM_W1 + NFC
SEM_QKV = SEM_W2 + NFC
SEM_WO = SEM_QKV + 3
SEM_OUT = SEM_WO + 8
NSEM = SEM_OUT + 1


def _kernel(x_hbm, mem0_ref, wq_hbm, wk_hbm, wv_hbm, wo_hbm, w1_hbm, b1_ref, w2_hbm, b2_ref,
            out_hbm,
            x_scr, xn_scr, acc_scr, out_scr, w1_scr, w2_scr, stage, wp_scr, wo_scr,
            ha_scr, hb_scr, qkva_scr, qkvb_scr, oa_scr, ob_scr, sems):
    def x_copy(b):
        rows = pl.ds(pl.multiple_of(b * TB, TB), TB)
        return pltpu.make_async_copy(x_hbm.at[rows], x_scr.at[rows], sems.at[SEM_X + b])

    def w1_copy(c):
        return pltpu.make_async_copy(w1_hbm.at[:, pl.ds(pl.multiple_of(c * FC, FC), FC)], w1_scr.at[c], sems.at[SEM_W1 + c])

    def w2_copy(c):
        return pltpu.make_async_copy(w2_hbm.at[pl.ds(pl.multiple_of(c * FC, FC), FC)], w2_scr.at[c], sems.at[SEM_W2 + c])

    qkv_hbm = (wq_hbm, wk_hbm, wv_hbm)

    def qkv_copy(m):
        return pltpu.make_async_copy(qkv_hbm[m], stage.at[m], sems.at[SEM_QKV + m])

    def wo_copy(j):
        return pltpu.make_async_copy(wo_hbm.at[:, pl.ds(j * DH, DH)], wo_scr.at[j], sems.at[SEM_WO + j])

    for b in range(XPB):
        x_copy(b).start()
    w1_copy(0).start()
    w2_copy(0).start()
    for b in range(XPB, NB):
        x_copy(b).start()
    for c in range(1, NFC):
        w1_copy(c).start()
        w2_copy(c).start()
    for m in range(3):
        qkv_copy(m).start()
    for j in range(NP_O):
        wo_copy(j).start()

    def ffn_iter(it, with_relayout):
        c = it // NBB
        bb = it % NBB
        r0 = pl.multiple_of(bb * RB, RB)

        @pl.when(c == 0)
        def _():
            for k in range(XPB):
                x_copy(bb * XPB + k).wait()
            x = x_scr[pl.ds(r0, RB), :].astype(f32)
            mu = jnp.mean(x, axis=-1, keepdims=True)
            xc = x - mu
            var = jnp.mean(xc * xc, axis=-1, keepdims=True)
            xn_scr[pl.ds(r0, RB), :] = (xc * lax.rsqrt(var + EPS)).astype(bf16)
            acc_scr[pl.ds(r0, RB), :] = x + b2_ref[...].astype(f32)

        @pl.when(bb == 0)
        def _():
            w1_copy(c).wait()
            w2_copy(c).wait()

        xn = xn_scr[pl.ds(r0, RB), :]
        h1 = jnp.dot(xn, w1_scr[c], preferred_element_type=f32) + b1_ref[c].astype(f32)
        g = jax.nn.gelu(h1, approximate=True).astype(bf16)
        acc_scr[pl.ds(r0, RB), :] += jnp.dot(g, w2_scr[c], preferred_element_type=f32)
        if with_relayout:
            step0 = (it - N_IT1) * RSTEPS
            for k in range(RSTEPS):
                step = step0 + k
                m = step // (D // RCH)
                d0 = pl.multiple_of((step % (D // RCH)) * RCH, RCH)
                blk = stage[m, pl.ds(d0, RCH)]
                wp_scr[pl.ds(pl.multiple_of(m * H, H), H), pl.ds(d0, RCH), :] = jnp.transpose(blk, (1, 0, 2))

    def ffn_body1(it, carry):
        ffn_iter(it, False)
        return carry

    def ffn_body2(it, carry):
        ffn_iter(it, True)
        return carry

    lax.fori_loop(0, N_IT1, ffn_body1, 0)
    for m in range(3):
        qkv_copy(m).wait()
    lax.fori_loop(N_IT1, N_IT, ffn_body2, 0)
    for j in range(NP_O):
        wo_copy(j).wait()

    scale = DH ** -0.5
    qi = lax.broadcasted_iota(jnp.int32, (L, L), 0)
    kj = lax.broadcasted_iota(jnp.int32, (L, L), 1)

    def tok_a(pos):
        return jnp.where(pos < 16, pos + 16, jnp.where(pos < 32, pos - 16, pos - 32))

    def mem_a(pos):
        return (pos >= 16) & (pos < 24)

    mask_a = mem_a(qi) | mem_a(kj) | (tok_a(kj) <= tok_a(qi))
    mask_b = (qi >= SEG) | (kj >= SEG) | (kj <= qi)

    c_exp = scale * 1.4426950408889634

    def attention(qkv_ref, mask):
        q = qkv_ref[0:H]
        k = qkv_ref[H:2 * H]
        v = qkv_ref[2 * H:3 * H]
        sc = jnp.einsum('hqd,hkd->hqk', q, k, preferred_element_type=f32)
        sc = jnp.where(mask[None], sc, -1e9)
        m = jnp.max(sc, axis=-1, keepdims=True)
        e = jnp.exp2((sc - m) * c_exp)
        l = jnp.sum(e, axis=-1, keepdims=True)
        r0 = pl.reciprocal(l, approx=True)
        r = r0 * (2.0 - l * r0)
        p = (e * r).astype(bf16)
        return jnp.einsum('hqk,hkd->hqd', p, v, preferred_element_type=f32)

    ha_scr[16:24, :] = mem0_ref[...]
    hp = xn_scr[0:16, :]
    for p in range(3 * H):
        r = jnp.dot(hp, wp_scr[p], preferred_element_type=f32)
        qkva_scr[p, 32:40, :] = r[0:8].astype(bf16)

    def out_copy(t0):
        return pltpu.make_async_copy(out_scr.at[pl.ds(t0, 2 * SEG)], out_hbm.at[pl.ds(t0, 2 * SEG)], sems.at[SEM_OUT])

    def dseg_body(i, carry):
        t0 = pl.multiple_of(i * (2 * SEG), 2 * SEG)
        ha_scr[0:16, :] = xn_scr[pl.ds(pl.multiple_of(t0 + 16, 16), 16), :]
        ha_scr[24:32, :] = xn_scr[pl.ds(pl.multiple_of(t0 + 8, 8), 8), :]
        ha = ha_scr[...]
        for p in range(3 * H):
            qkva_scr[p, 0:32, :] = jnp.dot(ha, wp_scr[p], preferred_element_type=f32).astype(bf16)
        oa = attention(qkva_scr, mask_a)
        for hd in range(H):
            oh = oa[hd]
            oa_scr[:, hd * DH:(hd + 1) * DH] = oh[0:32].astype(bf16)
            ob_scr[40:48, hd * DH:(hd + 1) * DH] = oh[32:40].astype(bf16)
        o = oa_scr[...]
        for j in range(NP_O):
            cs = slice(j * DH, (j + 1) * DH)
            r = jnp.dot(o, wo_scr[j], preferred_element_type=f32)
            rb = pl.ds(pl.multiple_of(t0 + 16, 16), 16)
            out_scr[rb, cs] = (acc_scr[rb, cs] + r[0:16]).astype(bf16)
            hb_scr[32:40, cs] = r[16:24].astype(bf16)
            ra = pl.ds(pl.multiple_of(t0 + 8, 8), 8)
            out_scr[ra, cs] = (acc_scr[ra, cs] + r[24:32]).astype(bf16)
        hb_scr[0:32, :] = xn_scr[pl.ds(pl.multiple_of(t0 + 32, 32), 32), :]
        nxt = pl.multiple_of(jnp.minimum(t0 + 64, S - 8), 8)
        hb_scr[40:48, :] = xn_scr[pl.ds(nxt, 8), :]
        hb = hb_scr[...]
        for p in range(3 * H):
            r = jnp.dot(hb, wp_scr[p], preferred_element_type=f32).astype(bf16)
            qkvb_scr[p] = r[0:40]
            qkva_scr[p, 32:40, :] = r[40:48]
        ob = attention(qkvb_scr, mask_b)
        for hd in range(H):
            ob_scr[0:40, hd * DH:(hd + 1) * DH] = ob[hd].astype(bf16)
        o = ob_scr[...]
        for j in range(NP_O):
            cs = slice(j * DH, (j + 1) * DH)
            r = jnp.dot(o, wo_scr[j], preferred_element_type=f32)
            rc = pl.ds(pl.multiple_of(t0 + 32, 32), 32)
            out_scr[rc, cs] = (acc_scr[rc, cs] + r[0:32]).astype(bf16)
            ha_scr[16:24, cs] = r[32:40].astype(bf16)
            rl = pl.ds(t0, 8)
            out_scr[rl, cs] = (acc_scr[rl, cs] + r[40:48]).astype(bf16)
        out_copy(t0).start()
        return carry

    lax.fori_loop(0, S // (2 * SEG), dseg_body, 0)

    def wait_body(i, carry):
        out_copy(pl.multiple_of(i * (2 * SEG), 2 * SEG)).wait()
        return carry

    lax.fori_loop(0, S // (2 * SEG), wait_body, 0)


@jax.jit
def pallas_parallel_sum__memory_aug_recurrent_mem_tr__dense_activation_gelu__prompt_kernel(A_x, A_mem0, A_Wq, A_Wk, A_Wv, A_Wo, A_seg_len, B_x, B_w1, B_b1, B_w2, B_b2):
    del A_seg_len, B_x
    assert A_x.shape == (1, S, D) and A_mem0.shape == (1, MEM, D)
    assert A_Wq.shape == (D, H, DH) and A_Wo.shape == (H, DH, D)
    assert B_w1.shape == (D, FF) and B_w2.shape == (FF, D)
    x = A_x.reshape(S, D)
    mem0 = A_mem0.reshape(MEM, D)
    wo = A_Wo.reshape(H * DH, D)
    b1 = B_b1.reshape(NFC, 1, FC)
    b2 = B_b2.reshape(1, D)
    any_spec = pl.BlockSpec(memory_space=pl.ANY)
    vmem_spec = pl.BlockSpec(memory_space=pltpu.VMEM)
    out = pl.pallas_call(
        _kernel,
        out_shape=jax.ShapeDtypeStruct((S, D), bf16),
        in_specs=[any_spec, vmem_spec, any_spec, any_spec, any_spec, any_spec, any_spec, vmem_spec, any_spec, vmem_spec],
        out_specs=any_spec,
        scratch_shapes=[
            pltpu.VMEM((S, D), bf16),
            pltpu.VMEM((S, D), bf16),
            pltpu.VMEM((S, D), f32),
            pltpu.VMEM((S, D), bf16),
            pltpu.VMEM((NFC, D, FC), bf16),
            pltpu.VMEM((NFC, FC, D), bf16),
            pltpu.VMEM((3, D, H, DH), bf16),
            pltpu.VMEM((3 * H, D, DH), bf16),
            pltpu.VMEM((NP_O, H * DH, DH), bf16),
            pltpu.VMEM((32, D), bf16),
            pltpu.VMEM((48, D), bf16),
            pltpu.VMEM((3 * H, L, DH), bf16),
            pltpu.VMEM((3 * H, L, DH), bf16),
            pltpu.VMEM((32, H * DH), bf16),
            pltpu.VMEM((48, H * DH), bf16),
            pltpu.SemaphoreType.DMA((NSEM,)),
        ],
        compiler_params=pltpu.CompilerParams(
            vmem_limit_bytes=120 * 1024 * 1024,
        ),
    )(x, mem0, A_Wq, A_Wk, A_Wv, wo, B_w1, b1, B_w2, b2)
    return out.reshape(1, S, D)
```
